```python
import jax
import jax.numpy as jnp

def _softmax(x, axis=-1):
    return jax.nn.softmax(x, axis=axis)

def _gelu(x):
    return jax.nn.gelu(x, approximate=True)

def _silu(x):
    return jax.nn.silu(x)

def _sigmoid(x):
    return jax.nn.sigmoid(x)

def _layernorm(x, axis=-1, eps=1e-05):
    m = jnp.mean(x, axis=axis, keepdims=True)
    v = jnp.var(x, axis=axis, keepdims=True)
    return (x - m) / jnp.sqrt(v + eps)

def _scatter_add(tgt, idx, src, axis=0):
    return tgt.at[idx].add(src)

def _segment_sum(src, seg, n):
    return jax.ops.segment_sum(src, seg, n)

class _Rng:

    def __init__(self, key):
        self._k = key

    def _next(self):
        self._k, sub = jax.random.split(self._k)
        return sub

    def normal(self, shape):
        return jax.random.normal(self._next(), shape, dtype=jnp.bfloat16)

    def randint(self, lo, hi, shape):
        return jax.random.randint(self._next(), shape, lo, hi, dtype=jnp.int32)

    def uniform(self, shape, lo=0.0, hi=1.0):
        return jax.random.uniform(self._next(), shape, jnp.bfloat16, lo, hi)

    def permutation(self, n):
        return jax.random.permutation(self._next(), n)
kernel_name = 'adaLN_cond__ssm_conv_h3__mixer_s_mlp__prompt'

def setup_inputs():
    _rng = _Rng(jax.random.key(int.from_bytes(__import__("os").urandom(4), "little")))
    _w = lambda a: (lambda t: t.astype(jnp.bfloat16) if jnp.issubdtype(t.dtype, jnp.floating) else t)(jnp.asarray(a))

    def _A_setup():
        B, S, D = (1, 2048, 640)
        ks = 4
        return {'q': _w((lambda *s: _rng.normal(s) * 0.05)(B, S, D)), 'k': _w((lambda *s: _rng.normal(s) * 0.05)(B, S, D)), 'v': _w((lambda *s: _rng.normal(s) * 0.05)(B, S, D)), 'shift_k': _w((lambda *s: _rng.normal(s) * 0.05)(D, ks) * 0.5), 'ssm_k': _w((lambda *s: _rng.normal(s) * 0.05)(D, S) * (1.0 / S ** 0.5)), 'ssm_D': _w((lambda *s: _rng.normal(s) * 0.05)(D))}
    _A_in = _A_setup()

    def _B_setup():
        B, S, D, F = (1, 2048, 640, 1728)
        return {'x': _w((lambda *s: _rng.normal(s) * 0.05)(B, S, D)), 'w1': _w((lambda *s: _rng.normal(s) * 0.05)(D, D) * D ** (-0.5)), 'w2': _w((lambda *s: _rng.normal(s) * 0.05)(D, D) * D ** (-0.5)), 'w3': _w((lambda *s: _rng.normal(s) * 0.05)(D, F) * D ** (-0.5)), 'w4': _w((lambda *s: _rng.normal(s) * 0.05)(F, D) * F ** (-0.5))}
    _B_in = _B_setup()
    return {'A_q': _A_in['q'], 'A_k': _A_in['k'], 'A_v': _A_in['v'], 'A_shift_k': _A_in['shift_k'], 'A_ssm_k': _A_in['ssm_k'], 'A_ssm_D': _A_in['ssm_D'], 'B_x': _B_in['x'], 'B_w1': _B_in['w1'], 'B_w2': _B_in['w2'], 'B_w3': _B_in['w3'], 'B_w4': _B_in['w4'], 'c': _w((lambda *s: _rng.normal(s) * 0.05)(1, 640)), 'w_mod': _w((lambda *s: _rng.normal(s) * 0.05)(640, 6 * 640) * 640 ** (-0.5))}

def reference(A_q, A_k, A_v, A_shift_k, A_ssm_k, A_ssm_D, B_x, B_w1, B_w2, B_w3, B_w4, c, w_mod):

    def _A_ref(q, k, v, shift_k, ssm_k, ssm_D):
        B, S, D = q.shape
        ks = shift_k.shape[-1]
        k_pad = jnp.pad(k, ((0, 0), (ks - 1, 0), (0, 0)))
        k_shift = jnp.zeros_like(k)
        for t in range(ks):
            k_shift = k_shift + k_pad[:, t:t + S, :] * shift_k[:, ks - 1 - t][None, None, :]
        kv = k_shift * v
        L = 2 * S
        kv_pad = jnp.pad(kv, ((0, 0), (0, S), (0, 0)))
        kf_pad = jnp.pad(ssm_k, ((0, 0), (0, S)))
        kv_f = (lambda x, axes=(-2, -1): jnp.fft.rfft2(x.astype(jnp.float32), axes=axes))(kv_pad[:, None, :, :], axes=(1, 2))
        kf_f = (lambda x, axes=(-2, -1): jnp.fft.rfft2(x.astype(jnp.float32), axes=axes))(kf_pad[:, None, :], axes=(1, 2))
        kf_f = (lambda x, *d: x.transpose(*d))(kf_f, 1, 2, 0)
        y_f = kv_f * kf_f[None, :, :, :]
        y = (lambda x, s, axes=(-2, -1): jnp.fft.irfft2(x, s=s, axes=axes).astype(jnp.bfloat16))(y_f, (1, L), axes=(1, 2))[:, 0, :S, :]
        y = y + kv * ssm_D[None, None, :]
        return q * y

    def _B_ref(x, w1, w2, w3, w4):
        B, S, D = x.shape
        h = _gelu(_layernorm(x, axis=-1) @ w1)
        c = D // 4
        g0 = jnp.pad(h[:, :, 0 * c:1 * c], ((0, 0), (1, 0), (0, 0)))[:, :S, :]
        g1 = jnp.pad(h[:, :, 1 * c:2 * c], ((0, 0), (0, 1), (0, 0)))[:, 1:, :]
        g2 = jnp.pad(h[:, :, 2 * c:3 * c], ((0, 0), (2, 0), (0, 0)))[:, :S, :]
        g3 = jnp.pad(h[:, :, 3 * c:], ((0, 0), (0, 2), (0, 0)))[:, 2:, :]
        hs = jnp.concatenate([g0, g1, g2, g3], axis=-1) @ w2
        x1 = x + hs
        h2 = _gelu(_layernorm(x1, axis=-1) @ w3) @ w4
        return x1 + h2
    x = A_q
    mod = (_silu(c) @ w_mod).reshape(c.shape[0], 6, 1, -1)
    sa, ca, ga, sb, cb, gb = (mod[:, 0].copy(), mod[:, 1].copy(), mod[:, 2].copy(), mod[:, 3].copy(), mod[:, 4].copy(), mod[:, 5].copy())
    h = _layernorm(x, axis=-1) * (1 + ca) + sa
    x = x + ga * _A_ref(h, A_k, A_v, A_shift_k, A_ssm_k, A_ssm_D)
    h = _layernorm(x, axis=-1) * (1 + cb) + sb
    x = x + gb * _B_ref(h, B_w1, B_w2, B_w3, B_w4)
    return x
```

```python
import numpy as np
import jax
import jax.numpy as jnp
import jax.experimental.pallas as pl
import jax.experimental.pallas.tpu as pltpu

S, D, F = 2048, 640, 1728
R = 256
T = 256
CH = 16
NT = S // R
NB = S // T
f32, bf16 = jnp.float32, jnp.bfloat16


def _dft_mats():
    f = np.arange(T)[:, None] + 0.5
    n = np.arange(T)[None, :]
    th = 2 * np.pi * f * n / (2 * T)
    fwd = np.concatenate([np.cos(th), -np.sin(th)], 0)
    th2 = (2 * np.pi * f * (n + T) / (2 * T)).T
    inv = np.concatenate([np.cos(th2), -np.sin(th2)], 1) / T
    return fwd.astype(np.float32), inv.astype(np.float32)


def _ln(x):
    m = jnp.mean(x, -1, keepdims=True)
    xc = x - m
    v = jnp.mean(xc * xc, -1, keepdims=True)
    return xc * jax.lax.rsqrt(v + 1e-5)


def _dot(a, b):
    return jnp.dot(a.astype(bf16), b, preferred_element_type=f32)


def _kernel(q_ref, k_ref, v_ref, sk_ref, kk_ref, sd_ref, w1_ref, w2_hbm, w3_hbm, w4_hbm,
            c_ref, wm_ref, fwd_ref, inv_ref, o_ref,
            mod, kcar, uprev, Ks, Ws, Y, xs, hbs, hs, w2, w3, w4, sems):
    i = pl.program_id(0)
    copies = [pltpu.make_async_copy(a, b, sems.at[n])
              for n, (a, b) in enumerate(((w2_hbm, w2), (w3_hbm, w3), (w4_hbm, w4)))]

    @pl.when(i == 0)
    def _():
        for cp in copies:
            cp.start()
        cc = c_ref[...].astype(f32)
        sc = jnp.broadcast_to(cc * jax.nn.sigmoid(cc), (8, D))
        mod[...] = _dot(sc, wm_ref[...])
        kcar[...] = jnp.zeros_like(kcar)
        uprev[...] = jnp.zeros_like(uprev)
        hs[0:8, :] = jnp.zeros((8, D), f32)
        hs[S + 8:S + 16, :] = jnp.zeros((8, D), f32)

    def m(j):
        return mod[0:1, j * D:(j + 1) * D]

    @pl.when(i < NT)
    def _():
        r0 = pl.multiple_of(i * R, R)
        kc = k_ref[...].astype(f32)
        kx = jnp.concatenate([kcar[...], kc], 0)
        kcar[...] = kc[R - 8:, :]
        sk = sk_ref[...].astype(f32)
        ksh = kc * sk[0:1]
        for j in range(1, 4):
            ksh = ksh + kx[8 - j:8 - j + R] * sk[j:j + 1]
        kv = ksh * v_ref[...].astype(f32)
        fwd = fwd_ref[...]
        par = jax.lax.broadcasted_iota(jnp.int32, (T, D), 0) & 1
        sg = (1 - 2 * par).astype(f32)
        ys = []
        for s in range(R // T):
            a = i * (R // T) + s
            U = jnp.dot(fwd, kv[s * T:(s + 1) * T].astype(bf16), preferred_element_type=f32)
            Ws[a, 0:T, :] = uprev[0:T, :] + sg * U[T:]
            Ws[a, T:, :] = uprev[T:, :] - sg * U[:T]
            uprev[...] = U
            Ks[a] = jax.lax.dot_general(fwd, kk_ref[:, s * T:(s + 1) * T],
                                        (((1,), (1,)), ((), ())), preferred_element_type=f32)

            def chunk(cix, _):
                c0 = pl.multiple_of(cix * CH, CH)
                re, im = pl.ds(c0, CH), pl.ds(T + c0, CH)

                def body(j, acc):
                    kr, ki = Ks[j, re, :], Ks[j, im, :]
                    wr, wi = Ws[a - j, re, :], Ws[a - j, im, :]
                    return (acc[0] + (kr * wr - ki * wi), acc[1] + (kr * wi + ki * wr))
                z = jnp.zeros((CH, D), f32)
                ar, ai = jax.lax.fori_loop(0, a + 1, body, (z, z))
                Y[re, :] = ar
                Y[im, :] = ai
                return 0
            jax.lax.fori_loop(0, T // CH, chunk, 0)
            ys.append(jnp.dot(inv_ref[...], Y[...].astype(bf16), preferred_element_type=f32))
        y = jnp.concatenate(ys, 0) + kv * sd_ref[...].astype(f32)
        x = q_ref[...].astype(f32)
        h = _ln(x) * (1 + m(1)) + m(0)
        x = x + m(2) * (h * y)
        xs[pl.ds(r0, R), :] = x
        hb = _ln(x) * (1 + m(4)) + m(3)
        hbs[pl.ds(r0, R), :] = hb
        hs[pl.ds(r0 + 8, R), :] = jax.nn.gelu(_dot(_ln(hb), w1_ref[...]), approximate=True)

    @pl.when(i == 1)
    def _():
        for cp in copies:
            cp.wait()

    @pl.when(i > 0)
    def _():
        r0 = pl.multiple_of((i - 1) * R, R)
        hw = hs[pl.ds(r0, R + 16), :]
        col = jax.lax.broadcasted_iota(jnp.int32, (R, D), 1)
        c = D // 4
        g = jnp.where(col < c, hw[7:7 + R],
                      jnp.where(col < 2 * c, hw[9:9 + R],
                                jnp.where(col < 3 * c, hw[6:6 + R], hw[10:10 + R])))
        x1 = hbs[pl.ds(r0, R), :] + _dot(g, w2[...])
        t = jax.nn.gelu(jax.lax.dot_general(_ln(x1).astype(bf16), w3[...], (((1,), (1,)), ((), ())), preferred_element_type=f32), approximate=True)
        b = x1 + _dot(t, w4[...])
        o_ref[...] = (xs[pl.ds(r0, R), :] + m(5) * b).astype(o_ref.dtype)


@jax.jit
def pallas_adaLN_cond__ssm_conv_h3__mixer_s_mlp__prompt_kernel(
    A_q, A_k, A_v, A_shift_k, A_ssm_k, A_ssm_D, B_x, B_w1, B_w2, B_w3, B_w4, c, w_mod,
):
    fwd, inv = _dft_mats()
    row = pl.BlockSpec((R, D), lambda i: (jnp.minimum(i, NT - 1), 0))
    full = lambda shp: pl.BlockSpec(shp, lambda i: (0,) * len(shp))
    hbm = pl.BlockSpec(memory_space=pl.ANY)
    out = pl.pallas_call(
        _kernel,
        grid=(NT + 1,),
        in_specs=[row, row, row, full((4, D)),
                  pl.BlockSpec((D, R), lambda i: (0, jnp.minimum(i, NT - 1))),
                  full((1, D)), full((D, D)), hbm, hbm, hbm,
                  full((1, D)), full((D, 6 * D)), full((2 * T, T)), full((T, 2 * T))],
        out_specs=pl.BlockSpec((R, D), lambda i: (jnp.maximum(i - 1, 0), 0)),
        out_shape=jax.ShapeDtypeStruct((S, D), bf16),
        scratch_shapes=[
            pltpu.VMEM((8, 6 * D), f32), pltpu.VMEM((8, D), f32), pltpu.VMEM((2 * T, D), f32),
            pltpu.VMEM((NB, 2 * T, D), f32), pltpu.VMEM((NB, 2 * T, D), f32),
            pltpu.VMEM((2 * T, D), f32),
            pltpu.VMEM((S, D), f32), pltpu.VMEM((S, D), f32), pltpu.VMEM((S + 16, D), f32),
            pltpu.VMEM((D, D), bf16), pltpu.VMEM((F, D), bf16), pltpu.VMEM((F, D), bf16),
            pltpu.SemaphoreType.DMA((3,)),
        ],
        compiler_params=pltpu.CompilerParams(
            dimension_semantics=("arbitrary",), vmem_limit_bytes=100 * 1024 * 1024),
    )(A_q[0], A_k[0], A_v[0], A_shift_k.T, A_ssm_k, A_ssm_D[None], B_w1, B_w2, B_w3.T, B_w4,
      c, w_mod, jnp.asarray(fwd, bf16), jnp.asarray(inv, bf16))
    return out[None]
```

```python
import numpy as np
import jax
import jax.numpy as jnp
import jax.experimental.pallas as pl
import jax.experimental.pallas.tpu as pltpu

S, D, F = 2048, 640, 1728
R = 256
T = 256
CH = 16
NT = S // R
NB = S // T
f32, bf16 = jnp.float32, jnp.bfloat16


def _dft_mats():
    f = np.arange(T)[:, None] + 0.5
    n = np.arange(T)[None, :]
    th = 2 * np.pi * f * n / (2 * T)
    fwd = np.concatenate([np.cos(th), -np.sin(th)], 0)
    th2 = (2 * np.pi * f * (n + T) / (2 * T)).T
    inv = np.concatenate([np.cos(th2), -np.sin(th2)], 1) / T
    return fwd.astype(np.float32), inv.astype(np.float32)


def _ln(x):
    m = jnp.mean(x, -1, keepdims=True)
    xc = x - m
    v = jnp.mean(xc * xc, -1, keepdims=True)
    return xc * jax.lax.rsqrt(v + 1e-5)


def _dot(a, b):
    return jnp.dot(a.astype(bf16), b, preferred_element_type=f32)


def _kernel(q_ref, k_ref, v_ref, sk_ref, kk_ref, sd_ref, w1_ref, w2_hbm, w3_hbm, w4_hbm,
            c_ref, wm_hbm, fwd_ref, inv_ref, o_ref,
            mod, kcar, uprev, Ks, Ws, Y, xs, hbs, hs, wm, w2, w3, w4, sems):
    i = pl.program_id(0)
    copies = [pltpu.make_async_copy(a, b, sems.at[n])
              for n, (a, b) in enumerate(((wm_hbm, wm), (w2_hbm, w2), (w3_hbm, w3), (w4_hbm, w4)))]

    @pl.when(i == 0)
    def _():
        for cp in copies:
            cp.start()
        kcar[...] = jnp.zeros_like(kcar)
        uprev[...] = jnp.zeros_like(uprev)
        hs[0:8, :] = jnp.zeros((8, D), f32)
        hs[S + 8:S + 16, :] = jnp.zeros((8, D), f32)

    def m(j):
        return mod[0:1, j * D:(j + 1) * D]

    @pl.when(i < NT)
    def _():
        r0 = pl.multiple_of(i * R, R)
        kc = k_ref[...].astype(f32)
        kx = jnp.concatenate([kcar[...], kc], 0)
        kcar[...] = kc[R - 8:, :]
        sk = sk_ref[...].astype(f32)
        ksh = kc * sk[0:1]
        for j in range(1, 4):
            ksh = ksh + kx[8 - j:8 - j + R] * sk[j:j + 1]
        kv = ksh * v_ref[...].astype(f32)
        fwd = fwd_ref[...]
        par = jax.lax.broadcasted_iota(jnp.int32, (T, D), 0) & 1
        sg = (1 - 2 * par).astype(f32)
        ys = []
        for s in range(R // T):
            a = i * (R // T) + s
            U = jnp.dot(fwd, kv[s * T:(s + 1) * T].astype(bf16), preferred_element_type=f32)
            Ws[a, 0:T, :] = uprev[0:T, :] + sg * U[T:]
            Ws[a, T:, :] = uprev[T:, :] - sg * U[:T]
            uprev[...] = U
            Ks[a] = jax.lax.dot_general(fwd, kk_ref[:, s * T:(s + 1) * T],
                                        (((1,), (1,)), ((), ())), preferred_element_type=f32)

            def accumulate(a):
                def chunk(cix, _):
                    c0 = pl.multiple_of(cix * CH, CH)
                    re, im = pl.ds(c0, CH), pl.ds(T + c0, CH)
                    ar = ai = None
                    for j in range(a + 1):
                        kr, ki = Ks[j, re, :], Ks[j, im, :]
                        wr, wi = Ws[a - j, re, :], Ws[a - j, im, :]
                        pr, pi = kr * wr - ki * wi, kr * wi + ki * wr
                        ar, ai = (pr, pi) if ar is None else (ar + pr, ai + pi)
                    Y[re, :] = ar
                    Y[im, :] = ai
                    return 0
                jax.lax.fori_loop(0, T // CH, chunk, 0)
            for n in range(NB):
                pl.when(a == n)(lambda n=n: accumulate(n))
            ys.append(jnp.dot(inv_ref[...], Y[...].astype(bf16), preferred_element_type=f32))
        y = jnp.concatenate(ys, 0) + kv * sd_ref[...].astype(f32)

        @pl.when(i == 0)
        def _():
            copies[0].wait()
            cc = c_ref[...].astype(f32)
            sc = jnp.broadcast_to(cc * jax.nn.sigmoid(cc), (8, D))
            mod[...] = _dot(sc, wm[...])

        x = q_ref[...].astype(f32)
        h = _ln(x) * (1 + m(1)) + m(0)
        x = x + m(2) * (h * y)
        xs[pl.ds(r0, R), :] = x
        hb = _ln(x) * (1 + m(4)) + m(3)
        hbs[pl.ds(r0, R), :] = hb
        hs[pl.ds(r0 + 8, R), :] = jax.nn.gelu(_dot(_ln(hb), w1_ref[...]), approximate=True)

    @pl.when(i == 1)
    def _():
        for cp in copies[1:]:
            cp.wait()

    @pl.when(i > 0)
    def _():
        r0 = pl.multiple_of((i - 1) * R, R)
        hw = hs[pl.ds(r0, R + 16), :]
        col = jax.lax.broadcasted_iota(jnp.int32, (R, D), 1)
        c = D // 4
        g = jnp.where(col < c, hw[7:7 + R],
                      jnp.where(col < 2 * c, hw[9:9 + R],
                                jnp.where(col < 3 * c, hw[6:6 + R], hw[10:10 + R])))
        x1 = hbs[pl.ds(r0, R), :] + _dot(g, w2[...])
        t = jax.nn.gelu(jax.lax.dot_general(_ln(x1).astype(bf16), w3[...], (((1,), (1,)), ((), ())), preferred_element_type=f32), approximate=True)
        b = x1 + _dot(t, w4[...])
        o_ref[...] = (xs[pl.ds(r0, R), :] + m(5) * b).astype(o_ref.dtype)


@jax.jit
def pallas_adaLN_cond__ssm_conv_h3__mixer_s_mlp__prompt_kernel(
    A_q, A_k, A_v, A_shift_k, A_ssm_k, A_ssm_D, B_x, B_w1, B_w2, B_w3, B_w4, c, w_mod,
):
    fwd, inv = _dft_mats()
    row = pl.BlockSpec((R, D), lambda i: (jnp.minimum(i, NT - 1), 0))
    full = lambda shp: pl.BlockSpec(shp, lambda i: (0,) * len(shp))
    hbm = pl.BlockSpec(memory_space=pl.ANY)
    out = pl.pallas_call(
        _kernel,
        grid=(NT + 1,),
        in_specs=[row, row, row, full((4, D)),
                  pl.BlockSpec((D, R), lambda i: (0, jnp.minimum(i, NT - 1))),
                  full((1, D)), full((D, D)), hbm, hbm, hbm,
                  full((1, D)), hbm, full((2 * T, T)), full((T, 2 * T))],
        out_specs=pl.BlockSpec((R, D), lambda i: (jnp.maximum(i - 1, 0), 0)),
        out_shape=jax.ShapeDtypeStruct((S, D), bf16),
        scratch_shapes=[
            pltpu.VMEM((8, 6 * D), f32), pltpu.VMEM((8, D), f32), pltpu.VMEM((2 * T, D), f32),
            pltpu.VMEM((NB, 2 * T, D), f32), pltpu.VMEM((NB, 2 * T, D), f32),
            pltpu.VMEM((2 * T, D), f32),
            pltpu.VMEM((S, D), f32), pltpu.VMEM((S, D), f32), pltpu.VMEM((S + 16, D), f32),
            pltpu.VMEM((D, 6 * D), bf16),
            pltpu.VMEM((D, D), bf16), pltpu.VMEM((F, D), bf16), pltpu.VMEM((F, D), bf16),
            pltpu.SemaphoreType.DMA((4,)),
        ],
        compiler_params=pltpu.CompilerParams(
            dimension_semantics=("arbitrary",), vmem_limit_bytes=100 * 1024 * 1024),
    )(A_q[0], A_k[0], A_v[0], A_shift_k.T, A_ssm_k, A_ssm_D[None], B_w1, B_w2, B_w3.T, B_w4,
      c, w_mod, jnp.asarray(fwd, bf16), jnp.asarray(inv, bf16))
    return out[None]
```

```python
import functools
import numpy as np
import jax
import jax.numpy as jnp
import jax.experimental.pallas as pl
import jax.experimental.pallas.tpu as pltpu

S, D, F = 2048, 640, 1728
R = 256
T = 256
CH = 16
RB = 32
FC = 256
NT = S // R
NB = S // T
f32, bf16 = jnp.float32, jnp.bfloat16


def _dft_mats():
    f = np.arange(T)[:, None] + 0.5
    n = np.arange(T)[None, :]
    th = 2 * np.pi * f * n / (2 * T)
    fwd = np.concatenate([np.cos(th), -np.sin(th)], 0)
    th2 = (2 * np.pi * f * (n + T) / (2 * T)).T
    inv = np.concatenate([np.cos(th2), -np.sin(th2)], 1) / T
    return fwd.astype(np.float32), inv.astype(np.float32)


def _ln(x):
    m = jnp.mean(x, -1, keepdims=True)
    xc = x - m
    v = jnp.mean(xc * xc, -1, keepdims=True)
    return xc * jax.lax.rsqrt(v + 1e-5)


def _dot(a, b):
    return jnp.dot(a.astype(bf16), b, preferred_element_type=f32)


def _kernel(q_ref, k_ref, v_ref, sk_ref, kk_ref, sd_ref, w1_ref, w2_hbm, w3_hbm, w4_hbm,
            c_ref, wm_hbm, fwd_ref, inv_ref, o_ref,
            mod, kcar, uprev, Ks, Ws, Y, kvs, xs, hbs, hs, wm, w2, w3, w4, sems):
    i = pl.program_id(0)
    copies = [pltpu.make_async_copy(a, b, sems.at[n])
              for n, (a, b) in enumerate(((wm_hbm, wm), (w2_hbm, w2), (w3_hbm, w3), (w4_hbm, w4)))]

    def m(j):
        return mod[0:1, j * D:(j + 1) * D]

    def phase_a(a):
        kc = k_ref[...].astype(f32)
        prev = kcar[...]
        kx = jnp.concatenate([prev, kc], 0)
        kcar[...] = kc[R - 8:, :]
        sk = sk_ref[...].astype(f32)
        ksh = kc * sk[0:1]
        for j in range(1, 4):
            ksh = ksh + kx[8 - j:8 - j + R] * sk[j:j + 1]
        kv = ksh * v_ref[...].astype(f32)
        kvs[...] = kv * sd_ref[...].astype(f32)
        fwd = fwd_ref[...]
        yield
        Ks[a] = jax.lax.dot_general(fwd, kk_ref[...], (((1,), (1,)), ((), ())),
                                    preferred_element_type=f32)
        yield
        U = jnp.dot(fwd, kv.astype(bf16), preferred_element_type=f32)
        par = jax.lax.broadcasted_iota(jnp.int32, (T, D), 0) & 1
        sg = (1 - 2 * par).astype(f32)
        Ws[a] = jnp.concatenate([uprev[0:T, :] + sg * U[T:], uprev[T:, :] - sg * U[:T]], 0)
        uprev[...] = U
        yield

        def accumulate(n):
            def chunk(cix, _):
                c0 = pl.multiple_of(cix * CH, CH)
                re, im = pl.ds(c0, CH), pl.ds(T + c0, CH)
                ar = ai = None
                for j in range(n + 1):
                    kr, ki = Ks[j, re, :], Ks[j, im, :]
                    wr, wi = Ws[n - j, re, :], Ws[n - j, im, :]
                    pr, pi = kr * wr - ki * wi, kr * wi + ki * wr
                    ar, ai = (pr, pi) if ar is None else (ar + pr, ai + pi)
                Y[re, :] = ar.astype(bf16)
                Y[im, :] = ai.astype(bf16)
                return 0
            jax.lax.fori_loop(0, T // CH, chunk, 0)
        for n in range(NB):
            pl.when(a == n)(functools.partial(accumulate, n))

    def phase_b(a):
        y = jnp.dot(inv_ref[...], Y[...], preferred_element_type=f32)
        yield
        ls = []
        for r in range(0, R, RB):
            rows = slice(r, r + RB)
            x = q_ref[rows, :].astype(f32)
            h = _ln(x) * (1 + m(1)) + m(0)
            x = x + m(2) * (h * (y[rows] + kvs[rows, :]))
            xs[a % 3, rows, :] = x
            hb = _ln(x) * (1 + m(4)) + m(3)
            hbs[a % 3, rows, :] = hb
            ls.append(_ln(hb).astype(bf16))
            yield
        z = jnp.dot(jnp.concatenate(ls, 0), w1_ref[...], preferred_element_type=f32)
        yield
        for r in range(0, R, RB):
            hs[pl.ds(pl.multiple_of(a * R + 8 + r, 8), RB), :] = jax.nn.gelu(z[r:r + RB], approximate=True)
            yield

    def phase_c(a):
        hw = hs[pl.ds(pl.multiple_of(a * R, R), R + 16), :]
        col = jax.lax.broadcasted_iota(jnp.int32, (R, D), 1)
        c = D // 4
        g = jnp.where(col < c, hw[7:7 + R],
                      jnp.where(col < 2 * c, hw[9:9 + R],
                                jnp.where(col < 3 * c, hw[6:6 + R], hw[10:10 + R])))
        x1 = hbs[a % 3] + _dot(g, w2[...])
        yield
        l = _ln(x1).astype(bf16)
        yield
        b = x1
        for f0 in range(0, F, FC):
            f1 = min(f0 + FC, F)
            t = jax.lax.dot_general(l, w3[f0:f1, :], (((1,), (1,)), ((), ())),
                                    preferred_element_type=f32)
            yield
            b = b + _dot(jax.nn.gelu(t, approximate=True), w4[f0:f1, :])
            yield
        o_ref[...] = (xs[a % 3] + m(5) * b).astype(o_ref.dtype)

    def run(b_on, c_on):
        gens = []
        if c_on:
            gens.append((phase_c(i - 2), 3 + 2 * -(-F // FC)))
        if b_on:
            gens.append((phase_b(i), 3 + 2 * (R // RB)))
        n = max(l for _, l in gens)
        done = [0] * len(gens)
        for t in range(1, n + 1):
            for gi, (g, l) in enumerate(gens):
                while done[gi] < -(-t * l // n):
                    next(g, None)
                    done[gi] += 1

    @pl.when(i == 0)
    def _():
        copies[0].start()
        kcar[...] = jnp.zeros_like(kcar)
        uprev[...] = jnp.zeros_like(uprev)
        hs[0:8, :] = jnp.zeros((8, D), f32)
        hs[S + 8:, :] = jnp.zeros((8, D), f32)

    @pl.when(i < NT)
    def _():
        for _ in phase_a(i):
            pass

    @pl.when(i == 0)
    def _():
        copies[0].wait()
        for cp in copies[1:]:
            cp.start()
        cc = c_ref[...].astype(f32)
        sc = jnp.broadcast_to(cc * jax.nn.sigmoid(cc), (8, D))
        mod[...] = _dot(sc, wm[...])

    @pl.when(i == 2)
    def _():
        for cp in copies[1:]:
            cp.wait()

    pl.when(i < 2)(lambda: run(True, False))
    pl.when((i >= 2) & (i < NT))(lambda: run(True, True))
    pl.when(i >= NT)(lambda: run(False, True))


@jax.jit
def pallas_adaLN_cond__ssm_conv_h3__mixer_s_mlp__prompt_kernel(
    A_q, A_k, A_v, A_shift_k, A_ssm_k, A_ssm_D, B_x, B_w1, B_w2, B_w3, B_w4, c, w_mod,
):
    fwd, inv = _dft_mats()
    row = pl.BlockSpec((R, D), lambda i: (jnp.minimum(i, NT - 1), 0))
    full = lambda shp: pl.BlockSpec(shp, lambda i: (0,) * len(shp))
    hbm = pl.BlockSpec(memory_space=pl.ANY)
    out = pl.pallas_call(
        _kernel,
        grid=(NT + 2,),
        in_specs=[row, row, row, full((4, D)),
                  pl.BlockSpec((D, R), lambda i: (0, jnp.minimum(i, NT - 1))),
                  full((1, D)), full((D, D)), hbm, hbm, hbm,
                  full((1, D)), hbm, full((2 * T, T)), full((T, 2 * T))],
        out_specs=pl.BlockSpec((R, D), lambda i: (jnp.maximum(i - 2, 0), 0)),
        out_shape=jax.ShapeDtypeStruct((S, D), bf16),
        scratch_shapes=[
            pltpu.VMEM((8, 6 * D), f32), pltpu.VMEM((8, D), f32), pltpu.VMEM((2 * T, D), f32),
            pltpu.VMEM((NB, 2 * T, D), f32), pltpu.VMEM((NB, 2 * T, D), f32),
            pltpu.VMEM((2 * T, D), bf16), pltpu.VMEM((R, D), f32),
            pltpu.VMEM((3, R, D), f32), pltpu.VMEM((3, R, D), f32), pltpu.VMEM((S + 16, D), f32),
            pltpu.VMEM((D, 6 * D), bf16),
            pltpu.VMEM((D, D), bf16), pltpu.VMEM((F, D), bf16), pltpu.VMEM((F, D), bf16),
            pltpu.SemaphoreType.DMA((4,)),
        ],
        compiler_params=pltpu.CompilerParams(
            dimension_semantics=("arbitrary",), vmem_limit_bytes=100 * 1024 * 1024),
    )(A_q[0], A_k[0], A_v[0], A_shift_k.T, A_ssm_k, A_ssm_D[None], B_w1, B_w2, B_w3.T, B_w4,
      c, w_mod, jnp.asarray(fwd, bf16), jnp.asarray(inv, bf16))
    return out[None]
```
